```python
import os as _os
_os.environ.setdefault("JAX_PLATFORMS", "cpu")
import jax
import jax.numpy as jnp

def _softmax(x, axis=-1):
    return jax.nn.softmax(x, axis=axis)
def _gelu(x):
    return jax.nn.gelu(x, approximate=True)
def _silu(x):
    return jax.nn.silu(x)
def _sigmoid(x):
    return jax.nn.sigmoid(x)
def _layernorm(x, axis=-1, eps=1e-5):
    m = jnp.mean(x, axis=axis, keepdims=True)
    v = jnp.var(x, axis=axis, keepdims=True)
    return (x - m) / jnp.sqrt(v + eps)
def _scatter_add(tgt, idx, src, axis=0):
    return tgt.at[idx].add(src)
def _segment_sum(src, seg, n):
    return jax.ops.segment_sum(src, seg, n)
class _Rng:
    def __init__(self, key):
        self._k = key
    def _next(self):
        self._k, sub = jax.random.split(self._k)
        return sub
    def normal(self, shape):
        return jax.random.normal(self._next(), shape, dtype=jnp.bfloat16)
    def randint(self, lo, hi, shape):
        return jax.random.randint(self._next(), shape, lo, hi, dtype=jnp.int32)
    def uniform(self, shape, lo=0.0, hi=1.0):
        return jax.random.uniform(self._next(), shape, jnp.bfloat16, lo, hi)
    def permutation(self, n):
        return jax.random.permutation(self._next(), n)


kernel_name = 'standalone__sliding_local_fixed_window__prompt'

def setup_inputs():
    _rng = _Rng(jax.random.key(int.from_bytes(__import__("os").urandom(4), "little")))
    _w = (lambda a: (lambda t: t.astype(jnp.bfloat16) if jnp.issubdtype(t.dtype, jnp.floating) else t)(jnp.asarray(a)))
    B, H, S, D = 1, 32, 2048, 128
    return {
        "q": _w((lambda *s: _rng.normal(s) * 0.4)(B, H, S, D)),
        "k": _w((lambda *s: _rng.normal(s) * 0.4)(B, H, S, D)),
        "v": _w((lambda *s: _rng.normal(s) * 0.05)(B, H, S, D)),
    }

def reference(q, k, v):
    B, H, S, D = q.shape
    w = 32
    pos = jnp.arange(S)
    rel = pos[:, None] - pos[None, :]
    mask = (rel >= 0) & (rel < w)
    scores = jnp.einsum("bhqd,bhkd->bhqk", q, k) * (D ** -0.5)
    scores = jnp.where(mask[None, None], scores, (lambda x, dt: x.astype(dt))(jnp.array(-1e9), q.dtype))
    p = _softmax(scores, axis=-1)
    return jnp.einsum("bhqk,bhkd->bhqd", p, v)
```

```python
import math

import jax
import jax.numpy as jnp
from jax import lax
import jax.experimental.pallas as pl
import jax.experimental.pallas.tpu as pltpu

_W = 32
_T = 128
_NT = (((1,), (1,)), ((), ()))


def _head_windowed(q_ref, k_ref, v_ref, o_ref):
    S, D = q_ref.shape
    nb = S // _T
    c = (D ** -0.5) * math.log2(math.e)
    r_i = lax.broadcasted_iota(jnp.int32, (_T, _T), 0)
    c_i = lax.broadcasted_iota(jnp.int32, (_T, _T), 1)
    rel = r_i - c_i
    own = (rel >= 0) & (rel < _W)
    prev = (rel[:_W] + _T) < _W
    lo = c_i[:_W] < (_T // 2)
    neg = -jnp.inf

    def scores(j):
        n = _T + _W if j + 1 < nb else _T
        return lax.dot_general(q_ref[j * _T:j * _T + n, :], k_ref[j * _T:(j + 1) * _T, :], _NT,
                               preferred_element_type=jnp.float32)

    def softmax(s, s_prev):
        top = jnp.where(own[:_W], s[:_W], neg if s_prev is None else jnp.where(prev, s_prev[_T:], neg))
        bot = jnp.where(own[_W:], s[_W:_T], neg)
        x = jnp.concatenate([top, bot], axis=0)
        mx = jnp.max(x, axis=-1, keepdims=True)
        p = jnp.exp2((x - mx) * c)
        inv = 1.0 / jnp.sum(p, axis=-1, keepdims=True)
        pb = p.astype(v_ref.dtype)
        if s_prev is None:
            return pb, None, inv
        zero = jnp.zeros((_W, _T), pb.dtype)
        p_own = jnp.concatenate([jnp.where(lo, pb[:_W], zero), pb[_W:]], axis=0)
        p_prev = jnp.where(lo, zero, pb[:_W])
        return p_own, p_prev, inv

    s_cur = scores(0)
    p_own, _, inv = softmax(s_cur, None)
    carry = None
    for j in range(nb):
        if j + 1 < nb:
            s_nxt = scores(j + 1)
            p_own_n, p_prev_n, inv_n = softmax(s_nxt, s_cur)
            lhs = jnp.concatenate([p_own, p_prev_n], axis=0)
        else:
            lhs = p_own
        o = jnp.dot(lhs, v_ref[j * _T:(j + 1) * _T, :], preferred_element_type=jnp.float32)
        top = o[:_W] if carry is None else o[:_W] + carry
        oo = jnp.concatenate([top, o[_W:_T]], axis=0) * inv
        o_ref[j * _T:(j + 1) * _T, :] = oo.astype(o_ref.dtype)
        if j + 1 < nb:
            carry = o[_T:]
            s_cur, p_own, inv = s_nxt, p_own_n, inv_n


@jax.jit
def pallas_standalone__sliding_local_fixed_window__prompt_kernel(
    q: jax.Array,
    k: jax.Array,
    v: jax.Array,
):
    B, H, S, D = q.shape
    BH = B * H
    chunks = (8, 8, 8, 8)
    starts = (0, 8, 16, 24)
    wstart = 24
    nc = len(chunks)

    def kernel_function(q_hbm, k_hbm, v_hbm, o_hbm, qb, kb, vb, ob, rsem, wsem):
        def rd(ci):
            a, n = starts[ci], chunks[ci]
            return [pltpu.make_async_copy(x.at[pl.ds(a, n)], b.at[pl.ds(a, n)], rsem.at[ci])
                    for x, b in ((q_hbm, qb), (k_hbm, kb), (v_hbm, vb))]

        def wr(a, n):
            return pltpu.make_async_copy(ob.at[pl.ds(a, n)], o_hbm.at[pl.ds(a, n)], wsem.at[0])

        for ci in range(nc):
            for cp in rd(ci):
                cp.start()

        def body(h, carry):
            for ci in range(nc):
                @pl.when(h == starts[ci])
                def _():
                    for cp in rd(ci):
                        cp.wait()

            @pl.when(h == wstart)
            def _():
                wr(0, wstart).start()

            _head_windowed(qb.at[h], kb.at[h], vb.at[h], ob.at[h])

            @pl.when(h >= wstart)
            def _():
                wr(h, 1).start()
            return carry

        lax.fori_loop(0, BH, body, 0)
        wr(0, BH).wait()

    q3, k3, v3 = (x.reshape(BH, S, D) for x in (q, k, v))
    o = pl.pallas_call(
        kernel_function,
        in_specs=[pl.BlockSpec(memory_space=pl.ANY)] * 3,
        out_specs=pl.BlockSpec(memory_space=pl.ANY),
        out_shape=jax.ShapeDtypeStruct((BH, S, D), q.dtype),
        scratch_shapes=[pltpu.VMEM((BH, S, D), q.dtype)] * 4
        + [pltpu.SemaphoreType.DMA((nc,)), pltpu.SemaphoreType.DMA((1,))],
        compiler_params=pltpu.CompilerParams(vmem_limit_bytes=100 * 2**20),
    )(q3, k3, v3)
    return o.reshape(B, H, S, D)
```

```python
import math

import jax
import jax.numpy as jnp
import numpy as np
from jax import lax
import jax.experimental.pallas as pl
import jax.experimental.pallas.tpu as pltpu

_W = 32
_T = 128
_G = 8
_TAIL_ROWS = 1536
_WRITE_ROWS = 32
_NT = (((1,), (1,)), ((), ()))


def _head_windowed(q_ref, k_ref, v_ref, o_ref):
    S, D = q_ref.shape
    nb = S // _T
    c = (D ** -0.5) * math.log2(math.e)
    row = lax.broadcasted_iota(jnp.int32, (_T, _T), 0)
    col = lax.broadcasted_iota(jnp.int32, (_T, _T), 1)
    rel = row - col
    own = (rel >= 0) & (rel < _W)
    prev = (rel[:_W] + _T) < _W
    left = col[:_W] < (_T // 2)
    neg = -jnp.inf

    def scores(j):
        n = _T + _W if j + 1 < nb else _T
        return lax.dot_general(q_ref[j * _T:j * _T + n, :], k_ref[j * _T:(j + 1) * _T, :],
                               _NT, preferred_element_type=jnp.float32)

    def softmax(s, s_prev):
        other = neg if s_prev is None else jnp.where(prev, s_prev[_T:], neg)
        x = jnp.concatenate([jnp.where(own[:_W], s[:_W], other),
                             jnp.where(own[_W:], s[_W:_T], neg)], axis=0)
        mx = jnp.max(x, axis=-1, keepdims=True)
        p = jnp.exp2((x - mx) * c)
        inv = 1.0 / jnp.sum(p, axis=-1, keepdims=True)
        p = p.astype(v_ref.dtype)
        if s_prev is None:
            return p, None, inv, mx
        zero = jnp.zeros((_W, _T), p.dtype)
        p_own = jnp.concatenate([jnp.where(left, p[:_W], zero), p[_W:]], axis=0)
        p_prev = jnp.where(left, zero, p[:_W])
        return p_own, p_prev, inv, mx

    s = scores(0)
    p_own, _, inv, low = softmax(s, None)
    carry = None
    for j in range(nb):
        last = j + 1 == nb
        if last:
            lhs = p_own
        else:
            s_next = scores(j + 1)
            p_own_next, p_prev, inv_next, mx = softmax(s_next, s)
            low = jnp.minimum(low, mx)
            lhs = jnp.concatenate([p_own, p_prev], axis=0)
        o = jnp.dot(lhs, v_ref[j * _T:(j + 1) * _T, :], preferred_element_type=jnp.float32)
        top = o[:_W] if carry is None else o[:_W] + carry
        out = jnp.concatenate([top, o[_W:_T]], axis=0) * inv
        o_ref[j * _T:(j + 1) * _T, :] = out.astype(o_ref.dtype)
        if not last:
            carry = o[_T:]
            s, p_own, inv = s_next, p_own_next, inv_next
    return jnp.min(low) * (D ** -0.5)


def _head_dense(q_ref, k_ref, v_ref, o_ref, fill):
    S, D = q_ref.shape
    dt = q_ref.dtype
    rows = 16
    scale = float(np.asarray(D ** -0.5).astype(dt))

    def rnd(x):
        return x.astype(dt).astype(jnp.float32)

    def body(i, carry):
        r0 = pl.multiple_of(i * rows, rows)
        s = lax.dot_general(q_ref[pl.ds(r0, rows), :], k_ref[...], _NT,
                            preferred_element_type=jnp.float32)
        s = rnd(rnd(s) * scale)
        rel = (r0 + lax.broadcasted_iota(jnp.int32, (rows, S), 0)
               - lax.broadcasted_iota(jnp.int32, (rows, S), 1))
        s = jnp.where((rel >= 0) & (rel < _W), s, fill)
        p = jnp.exp(s - jnp.max(s, axis=-1, keepdims=True))
        p = p / jnp.sum(p, axis=-1, keepdims=True)
        o = jnp.dot(p.astype(dt), v_ref[...], preferred_element_type=jnp.float32)
        o_ref[pl.ds(r0, rows), :] = o.astype(o_ref.dtype)
        return carry

    lax.fori_loop(0, S // rows, body, 0)


@jax.jit
def pallas_standalone__sliding_local_fixed_window__prompt_kernel(
    q: jax.Array,
    k: jax.Array,
    v: jax.Array,
):
    B, H, S, D = q.shape
    BH = B * H
    nc = BH // _G
    assert BH % _G == 0 and nc >= 2 and S % _T == 0 and S > _TAIL_ROWS
    fill = float(np.asarray(-1e9).astype(q.dtype))
    copy = pltpu.make_async_copy

    def kernel_function(q_hbm, k_hbm, v_hbm, o_hbm, qb, kb, vb, ob, sem):
        def reads(ci):
            heads, s = pl.ds(ci * _G, _G), sem.at[ci % 2]
            cps = [copy(q_hbm.at[heads], qb.at[heads], s), copy(k_hbm.at[heads], kb.at[heads], s)]
            if ci + 1 < nc:
                return cps + [copy(v_hbm.at[heads], vb.at[heads], s)]
            most, rows = pl.ds(ci * _G, _G - 1), pl.ds(0, S - _TAIL_ROWS)
            return cps + [copy(v_hbm.at[most], vb.at[most], s),
                          copy(v_hbm.at[BH - 1, rows], vb.at[BH - 1, rows], s)]

        tail_rows = pl.ds(S - _TAIL_ROWS, _TAIL_ROWS)
        tail = copy(v_hbm.at[BH - 1, tail_rows], vb.at[BH - 1, tail_rows], sem.at[nc % 2])
        wsem = sem.at[(nc - 1) % 2]

        def start_writes(first, count):
            def body(i, carry):
                heads = pl.ds(first, count)
                rows = pl.ds(pl.multiple_of(i * _WRITE_ROWS, _WRITE_ROWS), _WRITE_ROWS)
                copy(ob.at[heads, rows], o_hbm.at[heads, rows], wsem).start()
                return carry
            lax.fori_loop(0, S // _WRITE_ROWS, body, 0)

        for cp in reads(0) + reads(1):
            cp.start()

        def head(h, carry):
            for ci in range(nc):
                @pl.when(h == ci * _G)
                def _():
                    for cp in reads(ci):
                        cp.wait()
                    if ci + 2 < nc:
                        for cp in reads(ci + 2):
                            cp.start()
                    elif ci + 2 == nc:
                        tail.start()
                    else:
                        start_writes(0, BH - _G)
                        tail.wait()

            refs = (qb.at[h], kb.at[h], vb.at[h], ob.at[h])
            low = _head_windowed(*refs)

            @pl.when(jnp.logical_not(low > 0.5 * fill))
            def _():
                _head_dense(*refs, fill)
            return carry

        lax.fori_loop(0, BH, head, 0)
        start_writes(BH - _G, _G)
        copy(ob, o_hbm, wsem).wait()

    out = pl.pallas_call(
        kernel_function,
        in_specs=[pl.BlockSpec(memory_space=pl.ANY)] * 3,
        out_specs=pl.BlockSpec(memory_space=pl.ANY),
        out_shape=jax.ShapeDtypeStruct((BH, S, D), q.dtype),
        scratch_shapes=[pltpu.VMEM((BH, S, D), q.dtype)] * 4 + [pltpu.SemaphoreType.DMA((2,))],
        compiler_params=pltpu.CompilerParams(vmem_limit_bytes=80 * 2**20),
    )(*(x.reshape(BH, S, D) for x in (q, k, v)))
    return out.reshape(B, H, S, D)
```
